```python
import os as _os
_os.environ.setdefault("JAX_PLATFORMS", "cpu")
import jax
import jax.numpy as jnp

def _softmax(x, axis=-1):
    return jax.nn.softmax(x, axis=axis)
def _gelu(x):
    return jax.nn.gelu(x, approximate=True)
def _silu(x):
    return jax.nn.silu(x)
def _sigmoid(x):
    return jax.nn.sigmoid(x)
def _layernorm(x, axis=-1, eps=1e-5):
    m = jnp.mean(x, axis=axis, keepdims=True)
    v = jnp.var(x, axis=axis, keepdims=True)
    return (x - m) / jnp.sqrt(v + eps)
def _scatter_add(tgt, idx, src, axis=0):
    return tgt.at[idx].add(src)
def _segment_sum(src, seg, n):
    return jax.ops.segment_sum(src, seg, n)
class _Rng:
    def __init__(self, key):
        self._k = key
    def _next(self):
        self._k, sub = jax.random.split(self._k)
        return sub
    def normal(self, shape):
        return jax.random.normal(self._next(), shape, dtype=jnp.bfloat16)
    def randint(self, lo, hi, shape):
        return jax.random.randint(self._next(), shape, lo, hi, dtype=jnp.int32)
    def uniform(self, shape, lo=0.0, hi=1.0):
        return jax.random.uniform(self._next(), shape, jnp.bfloat16, lo, hi)
    def permutation(self, n):
        return jax.random.permutation(self._next(), n)


kernel_name = 'concat_heads__mha_block_cached__gqa_block_cached__near_ridge'

def setup_inputs():
    _rng = _Rng(jax.random.key(int.from_bytes(__import__("os").urandom(4), "little")))
    _w = (lambda a: (lambda t: t.astype(jnp.bfloat16) if jnp.issubdtype(t.dtype, jnp.floating) else t)(jnp.asarray(a)))
    def _A_setup():
        B, Sq, D = 8, 128, 512
        H, Sk, Dh = 32, 1024, 128
        return {
            "x": _w((lambda *s: _rng.normal(s) * 0.8)(B, Sq, D)),
            "k_cache": _w((lambda *s: _rng.normal(s) * 0.8)(B, H, Sk, Dh)),
            "v_cache": _w((lambda *s: _rng.normal(s) * 0.05)(B, H, Sk, Dh)),
            "wq": _w((lambda *s: _rng.normal(s) * 0.8)(D, H * Dh) * (D ** -0.5)),
            "wo": _w((lambda *s: _rng.normal(s) * 0.05)(H * Dh, D) * ((H * Dh) ** -0.5)),
        }
    _A_in = _A_setup()

    def _B_setup():
        B, Sq, D = 8, 128, 512
        Hq, Hkv, Sk, Dh = 32, 32, 1024, 128
        assert Hq % Hkv == 0, (Hq, Hkv)
        return {
            "x": _w((lambda *s: _rng.normal(s) * 0.8)(B, Sq, D)),
            "k_cache": _w((lambda *s: _rng.normal(s) * 0.8)(B, Hkv, Sk, Dh)),
            "v_cache": _w((lambda *s: _rng.normal(s) * 0.05)(B, Hkv, Sk, Dh)),
            "wq": _w((lambda *s: _rng.normal(s) * 0.8)(D, Hq * Dh) * (D ** -0.5)),
            "wo": _w((lambda *s: _rng.normal(s) * 0.05)(Hq * Dh, D) * ((Hq * Dh) ** -0.5)),
        }
    _B_in = _B_setup()

    return {
        "A_x": _A_in["x"],
        "A_k_cache": _A_in["k_cache"],
        "A_v_cache": _A_in["v_cache"],
        "A_wq": _A_in["wq"],
        "A_wo": _A_in["wo"],
        "B_x": _B_in["x"],
        "B_k_cache": _B_in["k_cache"],
        "B_v_cache": _B_in["v_cache"],
        "B_wq": _B_in["wq"],
        "B_wo": _B_in["wo"],
    }

def reference(A_x, A_k_cache, A_v_cache, A_wq, A_wo, B_x, B_k_cache, B_v_cache, B_wq, B_wo):
    def _A_ref(x, k_cache, v_cache, wq, wo):
        B, Sq, D = x.shape
        H, Dh = 32, 128
        q = (lambda x, *d: x.transpose(*d))((x @ wq).reshape(B, Sq, H, Dh), 0, 2, 1, 3)
        scores = jnp.einsum("bhqd,bhkd->bhqk", q, k_cache) * (Dh ** -0.5)
        p = _softmax(scores, axis=-1)
        o = jnp.einsum("bhqk,bhkd->bhqd", p, v_cache)
        return (lambda x, *d: x.transpose(*d))(o, 0, 2, 1, 3).reshape(B, Sq, H * Dh) @ wo

    def _B_ref(x, k_cache, v_cache, wq, wo):
        B, Sq, D = x.shape
        Hq, Dh = 32, 128
        Hkv = k_cache.shape[1]
        rep = Hq // Hkv
        q = (lambda x, *d: x.transpose(*d))((x @ wq).reshape(B, Sq, Hq, Dh), 0, 2, 1, 3)
        k = jnp.repeat(k_cache, rep, axis=1)
        v = jnp.repeat(v_cache, rep, axis=1)
        scores = jnp.einsum("bhqd,bhkd->bhqk", q, k) * (Dh ** -0.5)
        p = _softmax(scores, axis=-1)
        o = jnp.einsum("bhqk,bhkd->bhqd", p, v)
        return (lambda x, *d: x.transpose(*d))(o, 0, 2, 1, 3).reshape(B, Sq, Hq * Dh) @ wo

    a = _A_ref(A_x, A_k_cache, A_v_cache, A_wq, A_wo)
    b = _B_ref(B_x, B_k_cache, B_v_cache, B_wq, B_wo)
    return jnp.concatenate([a, b], axis=-1)
```

```python
import functools
import jax
import jax.numpy as jnp
import jax.experimental.pallas as pl
import jax.experimental.pallas.tpu as pltpu

NB = 4
NODMA = 0
ORDER = 'qvo'
LOG2E = 1.4426950408889634
NT = (((1,), (1,)), ((), ()))

def _ld(ref2d):
    return pltpu.bitcast(ref2d.bitcast(jnp.uint32)[...], jnp.bfloat16)

def _recip(l):
    r = pl.reciprocal(l, approx=True)
    return r * (2.0 - l * r)

def _kernel(ax, ak, av, awq, awo, bx, bk, bv, bwq, bwo, o_ref, acc, *, nb, Sq, Dh, D):
    h = pl.program_id(0)
    bi = pl.program_id(1)
    scale = (Dh ** -0.5) * LOG2E

    @pl.when((h == 0) & (bi == 0))
    def _():
        acc[...] = jnp.zeros_like(acc)

    brs = ((ax, ak, av, awq, awo), (bx, bk, bv, bwq, bwo))
    row0 = pl.multiple_of(bi * (nb * Sq), nb * Sq)
    qs = []
    for br, (x, k, v, wq, wo) in enumerate(brs):
        q = jnp.dot(x[pl.ds(row0, nb * Sq), :], wq[...], preferred_element_type=jnp.float32)
        qs.append((q * scale).astype(jnp.bfloat16))

    items = [(br, j) for br in range(2) for j in range(nb)]
    n = len(items)
    S = [None] * n
    O = [None] * n

    def do_qk(i):
        br, j = items[i]
        q = qs[br][j * Sq:(j + 1) * Sq]
        S[i] = jax.lax.dot_general(q, _ld(brs[br][1].at[j, 0]), NT, preferred_element_type=jnp.float32)

    def do_pv(i):
        br, j = items[i]
        s = S[i]
        m = jnp.max(s, axis=-1, keepdims=True)
        p = jnp.exp2(s - m)
        l = jnp.sum(p, axis=-1, keepdims=True)
        o = jnp.dot(p.astype(jnp.bfloat16), _ld(brs[br][2].at[j, 0]), preferred_element_type=jnp.float32)
        O[i] = (o * _recip(l)).astype(jnp.bfloat16)

    def do_o(i):
        br, j = items[i]
        row = pl.multiple_of(row0 + j * Sq, Sq)
        acc[pl.ds(row, Sq), br * D:(br + 1) * D] += jnp.dot(
            O[i], brs[br][4][...], preferred_element_type=jnp.float32)

    do_qk(0)
    for i in range(n):
        for c in ORDER:
            if c == 'q' and i + 1 < n: do_qk(i + 1)
            if c == 'o' and i >= 1: do_o(i - 1)
            if c == 'v': do_pv(i)
    do_o(n - 1)

    @pl.when((h == pl.num_programs(0) - 1) & (bi == pl.num_programs(1) - 1))
    def _():
        o_ref[...] = acc[...].astype(o_ref.dtype)


@jax.jit
def pallas_concat_heads__mha_block_cached__gqa_block_cached__near_ridge_kernel(
    A_x, A_k_cache, A_v_cache, A_wq, A_wo, B_x, B_k_cache, B_v_cache, B_wq, B_wo):
    B, Sq, D = A_x.shape
    _, H, Sk, Dh = A_k_cache.shape
    nb = NB
    ax = A_x.reshape(B * Sq, D)
    bx = B_x.reshape(B * Sq, D)
    x_spec = pl.BlockSpec((B * Sq, D), lambda h, bi: (0, 0))
    if NODMA:
        kv_spec = pl.BlockSpec((nb, 1, Sk, Dh), lambda h, bi: (0, 0, 0, 0))
    else:
        kv_spec = pl.BlockSpec((nb, 1, Sk, Dh), lambda h, bi: (bi, h, 0, 0))
    wq_spec = pl.BlockSpec((D, Dh), lambda h, bi: (0, h))
    wo_spec = pl.BlockSpec((Dh, D), lambda h, bi: (h, 0))
    specs = [x_spec, kv_spec, kv_spec, wq_spec, wo_spec]
    out = pl.pallas_call(
        functools.partial(_kernel, nb=nb, Sq=Sq, Dh=Dh, D=D),
        grid=(H, B // nb),
        in_specs=specs + specs,
        out_specs=pl.BlockSpec((B * Sq, 2 * D), lambda h, bi: (0, 0)),
        out_shape=jax.ShapeDtypeStruct((B * Sq, 2 * D), A_x.dtype),
        scratch_shapes=[pltpu.VMEM((B * Sq, 2 * D), jnp.float32)],
        compiler_params=pltpu.CompilerParams(
            dimension_semantics=("arbitrary", "arbitrary"),
            vmem_limit_bytes=100 * 1024 * 1024),
    )(ax, A_k_cache, A_v_cache, A_wq, A_wo, bx, B_k_cache, B_v_cache, B_wq, B_wo)
    return out.reshape(B, Sq, 2 * D)
```

```python
import functools
import jax
import jax.numpy as jnp
import jax.experimental.pallas as pl
import jax.experimental.pallas.tpu as pltpu

NB = 2
DEPTH = 3
ORDER = 'qvo'
NOBC = 1
NOCOMP = 0
DESC = 32 * 1024
LOG2E = 1.4426950408889634
NT = (((1,), (1,)), ((), ()))

def _ld(ref2d):
    return pltpu.bitcast(ref2d.bitcast(jnp.uint32)[...], jnp.bfloat16)

def _recip(l):
    r = pl.reciprocal(l, approx=True)
    return r * (2.0 - l * r)

def _kernel(ax, ak, av, awq, awo, bx, bk, bv, bwq, bwo, o_hbm,
            acc, kv, xb, wqb, wob, ob, kv_sem, x_sem, wq_sem, wo_sem, o_sem, *, nb, Sq, Sk, Dh, D, H, NBG):
    h = pl.program_id(0)
    bi = pl.program_id(1)
    T = H * NBG
    t = h * NBG + bi
    scale = (Dh ** -0.5) * LOG2E
    kv_hbm = (ak, av, bk, bv)
    x_hbm = (ax, bx)
    wq_hbm = (awq, bwq)
    wo_hbm = (awo, bwo)
    R = nb * Sq
    cnt = [0]
    def start(src, dst, sem):
        pltpu.make_async_copy(src, dst, sem).start(priority=cnt[0] % 2)
        cnt[0] += 1

    rc = DESC // (2 * Dh * nb)
    def issue_kv(step):
        hh = step // NBG
        bb = step % NBG
        slot = step % DEPTH
        for o in range(0, Sk, rc):
            for a in range(4):
                start(kv_hbm[a].at[pl.ds(bb * nb, nb), hh, pl.ds(o, rc)],
                      kv.at[slot, a, :, pl.ds(o, rc)], kv_sem.at[slot, a])

    def issue_x(g):
        xr = DESC // (2 * D)
        for o in range(g * R, (g + 1) * R, xr):
            for br in range(2):
                start(x_hbm[br].at[pl.ds(o, xr)], xb.at[br, pl.ds(o, xr)], x_sem.at[g])

    def issue_wq(hh):
        slot = hh % 2
        wr = DESC // (2 * Dh)
        for o in range(0, D, wr):
            for br in range(2):
                start(wq_hbm[br].at[pl.ds(o, wr), pl.ds(pl.multiple_of(hh * Dh, Dh), Dh)],
                      wqb.at[slot, br, pl.ds(o, wr)], wq_sem.at[slot])

    def issue_wo(hh):
        slot = hh % 2
        wr = DESC // (2 * D)
        for o in range(0, Dh, wr):
            for br in range(2):
                start(wo_hbm[br].at[pl.ds(pl.multiple_of(hh * Dh + o, wr), wr)],
                      wob.at[slot, br, pl.ds(o, wr)], wo_sem.at[slot])

    @pl.when(t == 0)
    def _():
        issue_x(0)
        issue_wq(jnp.int32(0))
        issue_kv(jnp.int32(0))
        issue_wo(jnp.int32(0))
        for d in range(1, DEPTH - 1):
            issue_x(d)
            issue_kv(jnp.int32(d))
        for g in range(DEPTH - 1, NBG):
            issue_x(g)
        acc[...] = jnp.zeros_like(acc)

    @pl.when(t + (DEPTH - 1) < T)
    def _():
        issue_kv(t + (DEPTH - 1))

    @pl.when((bi == 0) & (h + 1 < H))
    def _():
        issue_wq(h + 1)
        issue_wo(h + 1)

    row0 = pl.multiple_of(bi * R, R)
    ws = h % 2
    slot = t % DEPTH

    @pl.when(h == 0)
    def _():
        pltpu.make_async_copy(xb.at[:, pl.ds(row0, R)], xb.at[:, pl.ds(row0, R)], x_sem.at[bi]).wait()

    @pl.when(bi == 0)
    def _():
        pltpu.make_async_copy(wqb.at[ws], wqb.at[ws], wq_sem.at[ws]).wait()
        pltpu.make_async_copy(wob.at[ws], wob.at[ws], wo_sem.at[ws]).wait()

    for a in range(4):
        pltpu.make_async_copy(kv.at[slot, a], kv.at[slot, a], kv_sem.at[slot, a]).wait()

    items = [(br, j) for br in range(2) for j in range(nb)]
    n = len(items)

    if not NOCOMP:
        qs = []
        for br in range(2):
            q = jnp.dot(xb[br, pl.ds(row0, R), :], _ld(wqb.at[ws, br]), preferred_element_type=jnp.float32)
            qs.append((q * scale).astype(jnp.bfloat16))
        S = [None] * n
        O = [None] * n

        def do_qk(i):
            br, j = items[i]
            q = qs[br][j * Sq:(j + 1) * Sq]
            S[i] = jax.lax.dot_general(q, _ld(kv.at[slot, 2 * br, j]), NT, preferred_element_type=jnp.float32)

        def do_pv(i):
            br, j = items[i]
            s = S[i]
            m = jnp.max(s, axis=-1, keepdims=True)
            p = jnp.exp2(s - m)
            l = jnp.sum(p, axis=-1, keepdims=True)
            o = jnp.dot(p.astype(jnp.bfloat16), _ld(kv.at[slot, 2 * br + 1, j]), preferred_element_type=jnp.float32)
            O[i] = (o * _recip(l)).astype(jnp.bfloat16)

        def do_o(i):
            br, j = items[i]
            row = pl.multiple_of(row0 + j * Sq, Sq)
            acc[pl.ds(row, Sq), br * D:(br + 1) * D] += jnp.dot(
                O[i], wob[ws, br], preferred_element_type=jnp.float32)

        do_qk(0)
        for i in range(n):
            for c in ORDER:
                if c == 'q' and i + 1 < n: do_qk(i + 1)
                if c == 'o' and i >= 1: do_o(i - 1)
                if c == 'v': do_pv(i)
        do_o(n - 1)

    orows = DESC // (2 * 2 * D)
    @pl.when(h == H - 1)
    def _():
        ob[pl.ds(row0, R), :] = acc[pl.ds(row0, R), :].astype(ob.dtype)
        for o in range(0, R, orows):
            r = pl.multiple_of(row0 + o, orows)
            start(ob.at[pl.ds(r, orows)], o_hbm.at[pl.ds(r, orows)], o_sem)

    @pl.when(t == T - 1)
    def _():
        pltpu.make_async_copy(ob, ob, o_sem).wait()


@jax.jit
def pallas_concat_heads__mha_block_cached__gqa_block_cached__near_ridge_kernel(
    A_x, A_k_cache, A_v_cache, A_wq, A_wo, B_x, B_k_cache, B_v_cache, B_wq, B_wo):
    B, Sq, D = A_x.shape
    _, H, Sk, Dh = A_k_cache.shape
    nb = NB
    NBG = B // nb
    ax = A_x.reshape(B * Sq, D)
    bx = B_x.reshape(B * Sq, D)
    dt = A_x.dtype
    out = pl.pallas_call(
        functools.partial(_kernel, nb=nb, Sq=Sq, Sk=Sk, Dh=Dh, D=D, H=H, NBG=NBG),
        grid=(H, NBG),
        in_specs=[pl.BlockSpec(memory_space=pl.ANY)] * 10,
        out_specs=pl.BlockSpec(memory_space=pl.ANY),
        out_shape=jax.ShapeDtypeStruct((B * Sq, 2 * D), dt),
        scratch_shapes=[pltpu.VMEM((B * Sq, 2 * D), jnp.float32),
                        pltpu.VMEM((DEPTH, 4, nb, Sk, Dh), dt),
                        pltpu.VMEM((2, B * Sq, D), dt),
                        pltpu.VMEM((2, 2, D, Dh), dt),
                        pltpu.VMEM((2, 2, Dh, D), dt),
                        pltpu.VMEM((B * Sq, 2 * D), dt),
                        pltpu.SemaphoreType.DMA((DEPTH, 4)),
                        pltpu.SemaphoreType.DMA((NBG,)),
                        pltpu.SemaphoreType.DMA((2,)),
                        pltpu.SemaphoreType.DMA((2,)),
                        pltpu.SemaphoreType.DMA(())],
        compiler_params=pltpu.CompilerParams(
            dimension_semantics=("arbitrary", "arbitrary"),
            vmem_limit_bytes=100 * 1024 * 1024,
            disable_bounds_checks=bool(NOBC)),
    )(ax, A_k_cache, A_v_cache, A_wq, A_wo, bx, B_k_cache, B_v_cache, B_wq, B_wo)
    return out.reshape(B, Sq, 2 * D)
```

```python
import functools

import jax
import jax.numpy as jnp
import jax.experimental.pallas as pl
import jax.experimental.pallas.tpu as pltpu

NB = 4
DEPTH = 3
G = 4
KT = 6
DESC = 32 * 1024
LOG2E = 1.4426950408889634
NT = (((1,), (1,)), ((), ()))


def _recip(l):
    r = pl.reciprocal(l, approx=True)
    return r * (2.0 - l * r)


def _kernel(ax, ak, av, awq, awo, bx, bk, bv, bwq, bwo, o_hbm,
            acc, kv, xb, wqb, wob, ob, kv_sem, x_sem, w_sem, o_sem,
            *, nb, Sq, Sk, Dh, D, H, NQ):
    h = pl.program_id(0)
    c = pl.program_id(1)
    NC = 2 * NQ
    T = H * NC
    t = h * NC + c
    scale = (Dh ** -0.5) * LOG2E
    kv_hbm = ((ak, av), (bk, bv))
    x_hbm = (ax, bx)
    wq_hbm = (awq, bwq)
    wo_hbm = (awo, bwo)
    R = nb * Sq
    GS = G * NC
    NG = H // G
    cnt = [0]

    def start(src, dst, sem):
        pltpu.make_async_copy(src, dst, sem).start(priority=cnt[0] % 2)
        cnt[0] += 1

    def wait(buf, sem):
        pltpu.make_async_copy(buf, buf, sem).wait()

    def issue_kv(step, br, halves):
        rc = DESC // (2 * Dh * nb)
        hh = step // NC
        qq = (step % NC) // 2
        slot = step % DEPTH
        for half in halves:
            for o in range(half * Sk // 2, (half + 1) * Sk // 2, rc):
                for w in range(2):
                    start(kv_hbm[br][w].at[pl.ds(qq * nb, nb), hh, pl.ds(o, rc)],
                          kv.at[slot, :, w, pl.ds(o, rc)], kv_sem.at[slot])

    def issue_x(cc):
        br, qq = cc % 2, cc // 2
        xr = DESC // (2 * D)
        for o in range(qq * R, (qq + 1) * R, xr):
            start(x_hbm[br].at[pl.ds(o, xr)], xb.at[br, pl.ds(o, xr)], x_sem.at[cc])

    qr = D // GS
    orr = G * Dh // GS

    def issue_w(g, p):
        slot = g % 2
        for br in range(2):
            r = pl.multiple_of(p * qr, qr)
            start(wq_hbm[br].at[pl.ds(r, qr),
                                pl.ds(pl.multiple_of(g * (G * Dh), G * Dh), G * Dh)],
                  wqb.at[slot, br, pl.ds(r, qr)], w_sem.at[0, slot])
            r = pl.multiple_of(p * orr, orr)
            start(wo_hbm[br].at[pl.ds(pl.multiple_of(g * (G * Dh) + r, orr), orr)],
                  wob.at[slot, br, pl.ds(r, orr)], w_sem.at[1, slot])

    @pl.when(t == 0)
    def _():
        issue_x(0)
        for p in range(GS):
            issue_w(jnp.int32(0), jnp.int32(p))
        issue_kv(jnp.int32(0), 0, (0, 1))
        issue_x(1)
        issue_kv(jnp.int32(1), 1, (0, 1))
        for cc in range(2, NC):
            issue_x(cc)
        acc[...] = jnp.zeros_like(acc)

    g = h // G
    gp = t - g * GS

    @pl.when((g + 1 < NG) & (gp < GS // 2))
    def _():
        issue_w(g + 1, 2 * gp)
        issue_w(g + 1, 2 * gp + 1)

    br = c % 2
    qq = c // 2
    t0 = T - KT
    for b in range(2):
        @pl.when((br == 1 - b) & (t > t0) & (t + 1 < T))
        def _():
            issue_kv(t + 1, b, (1,))

    for b in range(2):
        @pl.when((br == b) & (t >= t0) & (t + 2 < T))
        def _():
            issue_kv(t + 2, b, (0,))

        @pl.when((br == b) & (t < t0))
        def _():
            issue_kv(t + 2, b, (0, 1))

    row0 = pl.multiple_of(qq * R, R)
    col0 = pl.multiple_of(br * D, D)
    ws = g % 2
    hl = pl.multiple_of((h - g * G) * Dh, Dh)
    slot = t % DEPTH

    @pl.when(h == 0)
    def _():
        wait(xb.at[br, pl.ds(row0, R)], x_sem.at[c])

    @pl.when(gp == 0)
    def _():
        wait(wqb.at[ws], w_sem.at[0, ws])
        wait(wob.at[ws], w_sem.at[1, ws])

    wait(kv.at[slot], kv_sem.at[slot])

    RL = (NQ - 1) * R

    @pl.when(t == T - 1)
    def _():
        start(ob.at[pl.ds(0, RL)], o_hbm.at[pl.ds(0, RL)], o_sem)
        start(ob.at[pl.ds(RL, R), pl.ds(0, D)], o_hbm.at[pl.ds(RL, R), pl.ds(0, D)], o_sem)

    def body(last):
        q_all = jnp.dot(xb[br, pl.ds(row0, R), :], wqb[ws, br, :, pl.ds(hl, Dh)],
                        preferred_element_type=jnp.float32)
        q_all = (q_all * scale).astype(jnp.bfloat16)
        S = [None] * nb
        O = [None] * nb

        def do_qk(j):
            q = q_all[j * Sq:(j + 1) * Sq]
            S[j] = jax.lax.dot_general(q, kv[slot, j, 0], NT,
                                       preferred_element_type=jnp.float32)

        def do_pv(j):
            s = S[j]
            m = jnp.max(s, axis=-1, keepdims=True)
            p = jnp.exp2(s - m)
            l = jnp.sum(p, axis=-1, keepdims=True)
            o = jnp.dot(p.astype(jnp.bfloat16), kv[slot, j, 1],
                        preferred_element_type=jnp.float32)
            O[j] = (o * _recip(l)).astype(jnp.bfloat16)

        def do_o(j):
            y = jnp.dot(O[j], wob[ws, br, pl.ds(hl, Dh), :],
                        preferred_element_type=jnp.float32)
            if last:
                row = RL + j * Sq
                ob[row:row + Sq, D:2 * D] = (acc[1, row:row + Sq, :] + y).astype(ob.dtype)
                start(ob.at[row:row + Sq, D:2 * D], o_hbm.at[row:row + Sq, D:2 * D], o_sem)
            else:
                row = pl.multiple_of(row0 + j * Sq, Sq)
                acc[br, pl.ds(row, Sq), :] += y

        do_qk(0)
        for i in range(nb):
            if i + 1 < nb:
                do_qk(i + 1)
            do_pv(i)
            if i >= 1:
                do_o(i - 1)
        do_o(nb - 1)

    @pl.when(t < T - 1)
    def _():
        body(False)

    @pl.when(t == T - 1)
    def _():
        body(True)

    @pl.when((h == H - 1) & (t < T - 1))
    def _():
        ob[pl.ds(row0, R), pl.ds(col0, D)] = acc[br, pl.ds(row0, R), :].astype(ob.dtype)

    @pl.when(t == T - 1)
    def _():
        wait(ob, o_sem)


@jax.jit
def pallas_concat_heads__mha_block_cached__gqa_block_cached__near_ridge_kernel(
    A_x: jax.Array,
    A_k_cache: jax.Array,
    A_v_cache: jax.Array,
    A_wq: jax.Array,
    A_wo: jax.Array,
    B_x: jax.Array,
    B_k_cache: jax.Array,
    B_v_cache: jax.Array,
    B_wq: jax.Array,
    B_wo: jax.Array,
):
    B, Sq, D = A_x.shape
    _, H, Sk, Dh = A_k_cache.shape
    assert B_k_cache.shape == A_k_cache.shape
    nb = NB
    NQ = B // nb
    dt = A_x.dtype
    out = pl.pallas_call(
        functools.partial(_kernel, nb=nb, Sq=Sq, Sk=Sk, Dh=Dh, D=D, H=H, NQ=NQ),
        grid=(H, 2 * NQ),
        in_specs=[pl.BlockSpec(memory_space=pl.ANY)] * 10,
        out_specs=pl.BlockSpec(memory_space=pl.ANY),
        out_shape=jax.ShapeDtypeStruct((B * Sq, 2 * D), dt),
        scratch_shapes=[
            pltpu.VMEM((2, B * Sq, D), jnp.float32),
            pltpu.VMEM((DEPTH, nb, 2, Sk, Dh), dt),
            pltpu.VMEM((2, B * Sq, D), dt),
            pltpu.VMEM((2, 2, D, G * Dh), dt),
            pltpu.VMEM((2, 2, G * Dh, D), dt),
            pltpu.VMEM((B * Sq, 2 * D), dt),
            pltpu.SemaphoreType.DMA((DEPTH,)),
            pltpu.SemaphoreType.DMA((2 * NQ,)),
            pltpu.SemaphoreType.DMA((2, 2)),
            pltpu.SemaphoreType.DMA(()),
        ],
        compiler_params=pltpu.CompilerParams(
            dimension_semantics=("arbitrary", "arbitrary"),
            vmem_limit_bytes=64 * 1024 * 1024,
            disable_bounds_checks=True),
    )(A_x.reshape(B * Sq, D), A_k_cache, A_v_cache, A_wq, A_wo,
      B_x.reshape(B * Sq, D), B_k_cache, B_v_cache, B_wq, B_wo)
    return out.reshape(B, Sq, 2 * D)
```

```python
import functools

import jax
import jax.numpy as jnp
import jax.experimental.pallas as pl
import jax.experimental.pallas.tpu as pltpu

NB = 4
DEPTH = 3
G = 4
KT = 6
DESC = 32 * 1024
QS = 4
LOG2E = 1.4426950408889634
NT = (((1,), (1,)), ((), ()))


def _recip(l):
    r = pl.reciprocal(l, approx=True)
    return r * (2.0 - l * r)


def _kernel(ax, ak, av, awq, awo, bx, bk, bv, bwq, bwo, o_hbm,
            acc, kv, xb, wqb, wob, ob, kv_sem, x_sem, w_sem, o_sem,
            *, nb, Sq, Sk, Dh, D, H, NQ):
    h = pl.program_id(0)
    c = pl.program_id(1)
    NC = 2 * NQ
    T = H * NC
    t = h * NC + c
    scale = (Dh ** -0.5) * LOG2E
    kv_hbm = ((ak, av), (bk, bv))
    x_hbm = (ax, bx)
    wq_hbm = (awq, bwq)
    wo_hbm = (awo, bwo)
    R = nb * Sq
    GS = G * NC
    NG = H // G
    cnt = [0]

    def start(src, dst, sem):
        pltpu.make_async_copy(src, dst, sem).start(priority=cnt[0] % 2)
        cnt[0] += 1

    def wait(buf, sem):
        pltpu.make_async_copy(buf, buf, sem).wait()

    def issue_kv(step, br, halves):
        rc = DESC // (2 * Dh * nb)
        hh = step // NC
        qq = (step % NC) // 2
        slot = step % DEPTH
        for half in halves:
            for o in range(half * Sk // 2, (half + 1) * Sk // 2, rc):
                for w in range(2):
                    start(kv_hbm[br][w].at[pl.ds(qq * nb, nb), hh, pl.ds(o, rc)],
                          kv.at[slot, :, w, pl.ds(o, rc)], kv_sem.at[slot])

    def issue_x(cc):
        br, qq = cc % 2, cc // 2
        xr = DESC // (2 * D)
        for o in range(qq * R, (qq + 1) * R, xr):
            start(x_hbm[br].at[pl.ds(o, xr)], xb.at[br, pl.ds(o, xr)], x_sem.at[cc])

    qr = D // QS // GS
    orr = G * Dh // GS

    def issue_w(g, p):
        slot = g % 2
        for br in range(2):
            r = pl.multiple_of(p * qr, qr)
            start(wq_hbm[br].at[:, pl.ds(r, qr),
                                pl.ds(pl.multiple_of(g * (G * Dh), G * Dh), G * Dh)],
                  wqb.at[slot, br, :, pl.ds(r, qr)], w_sem.at[0, slot])
            r = pl.multiple_of(p * orr, orr)
            start(wo_hbm[br].at[pl.ds(pl.multiple_of(g * (G * Dh) + r, orr), orr)],
                  wob.at[slot, br, pl.ds(r, orr)], w_sem.at[1, slot])

    @pl.when(t == 0)
    def _():
        issue_x(0)
        for p in range(GS):
            issue_w(jnp.int32(0), jnp.int32(p))
        issue_kv(jnp.int32(0), 0, (0, 1))
        issue_x(1)
        issue_kv(jnp.int32(1), 1, (0, 1))
        for cc in range(2, NC):
            issue_x(cc)
        acc[...] = jnp.zeros_like(acc)

    g = h // G
    gp = t - g * GS

    @pl.when((g + 1 < NG) & (gp < GS // 2))
    def _():
        issue_w(g + 1, 2 * gp)
        issue_w(g + 1, 2 * gp + 1)

    br = c % 2
    qq = c // 2
    t0 = T - KT
    for b in range(2):
        @pl.when((br == 1 - b) & (t > t0) & (t + 1 < T))
        def _():
            issue_kv(t + 1, b, (1,))

    for b in range(2):
        @pl.when((br == b) & (t >= t0) & (t + 2 < T))
        def _():
            issue_kv(t + 2, b, (0,))

        @pl.when((br == b) & (t < t0))
        def _():
            issue_kv(t + 2, b, (0, 1))

    row0 = pl.multiple_of(qq * R, R)
    col0 = pl.multiple_of(br * D, D)
    ws = g % 2
    hl = pl.multiple_of((h - g * G) * Dh, Dh)
    slot = t % DEPTH

    @pl.when(h == 0)
    def _():
        wait(xb.at[br, pl.ds(row0, R)], x_sem.at[c])

    @pl.when(gp == 0)
    def _():
        wait(wqb.at[ws], w_sem.at[0, ws])
        wait(wob.at[ws], w_sem.at[1, ws])

    wait(kv.at[slot], kv_sem.at[slot])

    RL = (NQ - 1) * R

    @pl.when(t == T - 1)
    def _():
        start(ob.at[pl.ds(0, RL)], o_hbm.at[pl.ds(0, RL)], o_sem)
        start(ob.at[pl.ds(RL, R), pl.ds(0, D)], o_hbm.at[pl.ds(RL, R), pl.ds(0, D)], o_sem)

    def body(last):
        wq_h = wqb[ws, br, :, :, pl.ds(hl, Dh)].reshape(D, Dh)
        q_all = jnp.dot(xb[br, pl.ds(row0, R), :], wq_h,
                        preferred_element_type=jnp.float32)
        q_all = (q_all * scale).astype(jnp.bfloat16)
        S = [None] * nb
        O = [None] * nb

        def do_qk(j):
            q = q_all[j * Sq:(j + 1) * Sq]
            S[j] = jax.lax.dot_general(q, kv[slot, j, 0], NT,
                                       preferred_element_type=jnp.float32)

        def do_pv(j):
            s = S[j]
            m = jnp.max(s, axis=-1, keepdims=True)
            p = jnp.exp2(s - m)
            l = jnp.sum(p, axis=-1, keepdims=True)
            o = jnp.dot(p.astype(jnp.bfloat16), kv[slot, j, 1],
                        preferred_element_type=jnp.float32)
            O[j] = (o * _recip(l)).astype(jnp.bfloat16)

        def do_o(j):
            y = jnp.dot(O[j], wob[ws, br, pl.ds(hl, Dh), :],
                        preferred_element_type=jnp.float32)
            if last:
                row = RL + j * Sq
                ob[row:row + Sq, D:2 * D] = (acc[1, row:row + Sq, :] + y).astype(ob.dtype)
                start(ob.at[row:row + Sq, D:2 * D], o_hbm.at[row:row + Sq, D:2 * D], o_sem)
            else:
                row = pl.multiple_of(row0 + j * Sq, Sq)
                acc[br, pl.ds(row, Sq), :] += y

        do_qk(0)
        for i in range(nb):
            if i + 1 < nb:
                do_qk(i + 1)
            do_pv(i)
            if i >= 1:
                do_o(i - 1)
        do_o(nb - 1)

    @pl.when(t < T - 1)
    def _():
        body(False)

    @pl.when(t == T - 1)
    def _():
        body(True)

    @pl.when((h == H - 1) & (t < T - 1))
    def _():
        ob[pl.ds(row0, R), pl.ds(col0, D)] = acc[br, pl.ds(row0, R), :].astype(ob.dtype)

    @pl.when(t == T - 1)
    def _():
        wait(ob, o_sem)


@jax.jit
def pallas_concat_heads__mha_block_cached__gqa_block_cached__near_ridge_kernel(
    A_x: jax.Array,
    A_k_cache: jax.Array,
    A_v_cache: jax.Array,
    A_wq: jax.Array,
    A_wo: jax.Array,
    B_x: jax.Array,
    B_k_cache: jax.Array,
    B_v_cache: jax.Array,
    B_wq: jax.Array,
    B_wo: jax.Array,
):
    B, Sq, D = A_x.shape
    _, H, Sk, Dh = A_k_cache.shape
    assert B_k_cache.shape == A_k_cache.shape
    nb = NB
    NQ = B // nb
    dt = A_x.dtype
    out = pl.pallas_call(
        functools.partial(_kernel, nb=nb, Sq=Sq, Sk=Sk, Dh=Dh, D=D, H=H, NQ=NQ),
        grid=(H, 2 * NQ),
        in_specs=[pl.BlockSpec(memory_space=pl.ANY)] * 10,
        out_specs=pl.BlockSpec(memory_space=pl.ANY),
        out_shape=jax.ShapeDtypeStruct((B * Sq, 2 * D), dt),
        scratch_shapes=[
            pltpu.VMEM((2, B * Sq, D), jnp.float32),
            pltpu.VMEM((DEPTH, nb, 2, Sk, Dh), dt),
            pltpu.VMEM((2, B * Sq, D), dt),
            pltpu.VMEM((2, 2, QS, D // QS, G * Dh), dt),
            pltpu.VMEM((2, 2, G * Dh, D), dt),
            pltpu.VMEM((B * Sq, 2 * D), dt),
            pltpu.SemaphoreType.DMA((DEPTH,)),
            pltpu.SemaphoreType.DMA((2 * NQ,)),
            pltpu.SemaphoreType.DMA((2, 2)),
            pltpu.SemaphoreType.DMA(()),
        ],
        compiler_params=pltpu.CompilerParams(
            dimension_semantics=("arbitrary", "arbitrary"),
            vmem_limit_bytes=64 * 1024 * 1024,
            disable_bounds_checks=True),
    )(A_x.reshape(B * Sq, D), A_k_cache, A_v_cache, A_wq.reshape(QS, D // QS, H * Dh), A_wo,
      B_x.reshape(B * Sq, D), B_k_cache, B_v_cache, B_wq.reshape(QS, D // QS, H * Dh), B_wo)
    return out.reshape(B, Sq, 2 * D)
```

```python
import functools

import jax
import jax.numpy as jnp
import jax.experimental.pallas as pl
import jax.experimental.pallas.tpu as pltpu

NB = 4
DEPTH = 3
G = 4
KT = 6
DESC = 32 * 1024
QS = 4
LOG2E = 1.4426950408889634
NT = (((1,), (1,)), ((), ()))


def _recip(l):
    r = pl.reciprocal(l, approx=True)
    return r * (2.0 - l * r)


def _kernel(ax, ak, av, awq, awo, bx, bk, bv, bwq, bwo, o_hbm,
            acc, kv, xb, wqb, wob, ob, kv_sem, x_sem, w_sem, o_sem,
            *, nb, Sq, Sk, Dh, D, H, NQ):
    h = pl.program_id(0)
    c = pl.program_id(1)
    NC = 2 * NQ
    T = H * NC
    t = h * NC + c
    scale = (Dh ** -0.5) * LOG2E
    kv_hbm = ((ak, av), (bk, bv))
    x_hbm = (ax, bx)
    wq_hbm = (awq, bwq)
    wo_hbm = (awo, bwo)
    R = nb * Sq
    GS = G * NC
    NG = H // G
    cnt = [0]

    def start(src, dst, sem):
        pltpu.make_async_copy(src, dst, sem).start(priority=cnt[0] % 2)
        cnt[0] += 1

    def wait(buf, sem):
        pltpu.make_async_copy(buf, buf, sem).wait()

    def issue_kv(step, br, halves):
        rc = DESC // (2 * Dh * nb)
        hh = step // NC
        qq = (step % NC) // 2
        slot = step % DEPTH
        for half in halves:
            for o in range(half * Sk // 2, (half + 1) * Sk // 2, rc):
                for w in range(2):
                    start(kv_hbm[br][w].at[pl.ds(qq * nb, nb), hh, pl.ds(o, rc)],
                          kv.at[slot, :, w, pl.ds(o, rc)], kv_sem.at[slot])

    def issue_x(cc):
        br, qq = cc % 2, cc // 2
        xr = DESC // (2 * D)
        for o in range(qq * R, (qq + 1) * R, xr):
            start(x_hbm[br].at[pl.ds(o, xr)], xb.at[br, pl.ds(o, xr)], x_sem.at[cc])

    qr = D // QS // GS
    orr = G * Dh // GS

    def issue_w(g, p):
        slot = g % 2
        for br in range(2):
            r = pl.multiple_of(p * qr, qr)
            start(wq_hbm[br].at[:, pl.ds(r, qr),
                                pl.ds(pl.multiple_of(g * (G * Dh), G * Dh), G * Dh)],
                  wqb.at[slot, br, :, pl.ds(r, qr)], w_sem.at[slot])
            r = pl.multiple_of(p * orr, orr)
            start(wo_hbm[br].at[pl.ds(pl.multiple_of(g * (G * Dh) + r, orr), orr)],
                  wob.at[slot, br, pl.ds(r, orr)], w_sem.at[2 + slot])

    @pl.when(t == 0)
    def _():
        issue_x(0)
        for p in range(GS):
            issue_w(jnp.int32(0), jnp.int32(p))
        issue_kv(jnp.int32(0), 0, (0, 1))
        issue_x(1)
        issue_kv(jnp.int32(1), 1, (0, 1))
        for cc in range(2, NC):
            issue_x(cc)
        acc[...] = jnp.zeros_like(acc)

    g = h // G
    gp = t - g * GS

    @pl.when((g + 1 < NG) & (gp < GS // 2))
    def _():
        issue_w(g + 1, 2 * gp)
        issue_w(g + 1, 2 * gp + 1)

    br = c % 2
    qq = c // 2
    t0 = T - KT
    for b in range(2):
        @pl.when((br == 1 - b) & (t > t0) & (t + 1 < T))
        def _():
            issue_kv(t + 1, b, (1,))

    for b in range(2):
        @pl.when((br == b) & (t >= t0) & (t + 2 < T))
        def _():
            issue_kv(t + 2, b, (0,))

        @pl.when((br == b) & (t < t0))
        def _():
            issue_kv(t + 2, b, (0, 1))

    row0 = pl.multiple_of(qq * R, R)
    col0 = pl.multiple_of(br * D, D)
    ws = g % 2
    hl = pl.multiple_of((h - g * G) * Dh, Dh)
    slot = t % DEPTH

    @pl.when(h == 0)
    def _():
        wait(xb.at[br, pl.ds(row0, R)], x_sem.at[c])

    @pl.when(gp == 0)
    def _():
        wait(wqb.at[ws], w_sem.at[ws])
        wait(wob.at[ws], w_sem.at[2 + ws])

    wait(kv.at[slot], kv_sem.at[slot])

    RL = (NQ - 1) * R

    @pl.when(t == T - 1)
    def _():
        start(ob.at[pl.ds(0, RL)], o_hbm.at[pl.ds(0, RL)], o_sem)
        start(ob.at[pl.ds(RL, R), pl.ds(0, D)], o_hbm.at[pl.ds(RL, R), pl.ds(0, D)], o_sem)

    def body(last):
        wq_h = wqb[ws, br, :, :, pl.ds(hl, Dh)].reshape(D, Dh)
        q_all = jnp.dot(xb[br, pl.ds(row0, R), :], wq_h,
                        preferred_element_type=jnp.float32)
        q_all = (q_all * scale).astype(jnp.bfloat16)
        S = [None] * nb
        O = [None] * nb

        def do_qk(j):
            q = q_all[j * Sq:(j + 1) * Sq]
            S[j] = jax.lax.dot_general(q, kv[slot, j, 0], NT,
                                       preferred_element_type=jnp.float32)

        def do_pv(j):
            s = S[j]
            m = jnp.max(s, axis=-1, keepdims=True)
            p = jnp.exp2(s - m)
            l = jnp.sum(p, axis=-1, keepdims=True)
            o = jnp.dot(p.astype(jnp.bfloat16), kv[slot, j, 1],
                        preferred_element_type=jnp.float32)
            O[j] = (o * _recip(l)).astype(jnp.bfloat16)

        def do_o(j):
            y = jnp.dot(O[j], wob[ws, br, pl.ds(hl, Dh), :],
                        preferred_element_type=jnp.float32)
            if last:
                row = RL + j * Sq
                ob[row:row + Sq, D:2 * D] = (acc[1, row:row + Sq, :] + y).astype(ob.dtype)
                start(ob.at[row:row + Sq, D:2 * D], o_hbm.at[row:row + Sq, D:2 * D], o_sem)
            else:
                row = pl.multiple_of(row0 + j * Sq, Sq)
                acc[br, pl.ds(row, Sq), :] += y

        do_qk(0)
        for i in range(nb):
            if i + 1 < nb:
                do_qk(i + 1)
            do_pv(i)
            if i >= 1:
                do_o(i - 1)
        do_o(nb - 1)

    @pl.when(t < T - 1)
    def _():
        body(False)

    @pl.when(t == T - 1)
    def _():
        body(True)

    @pl.when((h == H - 1) & (t < T - 1))
    def _():
        ob[pl.ds(row0, R), pl.ds(col0, D)] = acc[br, pl.ds(row0, R), :].astype(ob.dtype)

    @pl.when(t == T - 1)
    def _():
        wait(ob, o_sem)


@jax.jit
def pallas_concat_heads__mha_block_cached__gqa_block_cached__near_ridge_kernel(
    A_x: jax.Array,
    A_k_cache: jax.Array,
    A_v_cache: jax.Array,
    A_wq: jax.Array,
    A_wo: jax.Array,
    B_x: jax.Array,
    B_k_cache: jax.Array,
    B_v_cache: jax.Array,
    B_wq: jax.Array,
    B_wo: jax.Array,
):
    B, Sq, D = A_x.shape
    _, H, Sk, Dh = A_k_cache.shape
    assert B_k_cache.shape == A_k_cache.shape
    nb = NB
    NQ = B // nb
    dt = A_x.dtype
    out = pl.pallas_call(
        functools.partial(_kernel, nb=nb, Sq=Sq, Sk=Sk, Dh=Dh, D=D, H=H, NQ=NQ),
        grid=(H, 2 * NQ),
        in_specs=[pl.BlockSpec(memory_space=pl.ANY)] * 10,
        out_specs=pl.BlockSpec(memory_space=pl.ANY),
        out_shape=jax.ShapeDtypeStruct((B * Sq, 2 * D), dt),
        scratch_shapes=[
            pltpu.VMEM((2, B * Sq, D), jnp.float32),
            pltpu.VMEM((DEPTH, nb, 2, Sk, Dh), dt),
            pltpu.VMEM((2, B * Sq, D), dt),
            pltpu.VMEM((2, 2, QS, D // QS, G * Dh), dt),
            pltpu.VMEM((2, 2, G * Dh, D), dt),
            pltpu.VMEM((B * Sq, 2 * D), dt),
            pltpu.SemaphoreType.DMA((DEPTH,)),
            pltpu.SemaphoreType.DMA((2 * NQ,)),
            pltpu.SemaphoreType.DMA((4,)),
            pltpu.SemaphoreType.DMA(()),
        ],
        compiler_params=pltpu.CompilerParams(
            dimension_semantics=("arbitrary", "arbitrary"),
            vmem_limit_bytes=64 * 1024 * 1024,
            disable_bounds_checks=True),
    )(A_x.reshape(B * Sq, D), A_k_cache, A_v_cache, A_wq.reshape(QS, D // QS, H * Dh), A_wo,
      B_x.reshape(B * Sq, D), B_k_cache, B_v_cache, B_wq.reshape(QS, D // QS, H * Dh), B_wo)
    return out.reshape(B, Sq, 2 * D)
```
